```python
import os as _os
_os.environ.setdefault("JAX_PLATFORMS", "cpu")
import jax
import jax.numpy as jnp

def _softmax(x, axis=-1):
    return jax.nn.softmax(x, axis=axis)
def _gelu(x):
    return jax.nn.gelu(x, approximate=True)
def _silu(x):
    return jax.nn.silu(x)
def _sigmoid(x):
    return jax.nn.sigmoid(x)
def _layernorm(x, axis=-1, eps=1e-5):
    m = jnp.mean(x, axis=axis, keepdims=True)
    v = jnp.var(x, axis=axis, keepdims=True)
    return (x - m) / jnp.sqrt(v + eps)
def _scatter_add(tgt, idx, src, axis=0):
    return tgt.at[idx].add(src)
def _segment_sum(src, seg, n):
    return jax.ops.segment_sum(src, seg, n)
class _Rng:
    def __init__(self, key):
        self._k = key
    def _next(self):
        self._k, sub = jax.random.split(self._k)
        return sub
    def normal(self, shape):
        return jax.random.normal(self._next(), shape, dtype=jnp.bfloat16)
    def randint(self, lo, hi, shape):
        return jax.random.randint(self._next(), shape, lo, hi, dtype=jnp.int32)
    def uniform(self, shape, lo=0.0, hi=1.0):
        return jax.random.uniform(self._next(), shape, jnp.bfloat16, lo, hi)
    def permutation(self, n):
        return jax.random.permutation(self._next(), n)


kernel_name = 'concat_heads__gqa_block_cached__sliding_block_cached__decode'

def setup_inputs():
    _rng = _Rng(jax.random.key(int.from_bytes(__import__("os").urandom(4), "little")))
    _w = (lambda a: (lambda t: t.astype(jnp.bfloat16) if jnp.issubdtype(t.dtype, jnp.floating) else t)(jnp.asarray(a)))
    def _A_setup():
        B, Sq, D = 1, 1, 576
        Hq, Hkv, Sk, Dh = 32, 16, 8192, 128
        assert Hq % Hkv == 0, (Hq, Hkv)
        return {
            "x": _w((lambda *s: _rng.normal(s) * 0.8)(B, Sq, D)),
            "k_cache": _w((lambda *s: _rng.normal(s) * 0.8)(B, Hkv, Sk, Dh)),
            "v_cache": _w((lambda *s: _rng.normal(s) * 0.05)(B, Hkv, Sk, Dh)),
            "wq": _w((lambda *s: _rng.normal(s) * 0.8)(D, Hq * Dh) * (D ** -0.5)),
            "wo": _w((lambda *s: _rng.normal(s) * 0.05)(Hq * Dh, D) * ((Hq * Dh) ** -0.5)),
        }
    _A_in = _A_setup()

    def _B_setup():
        B, Sq, D = 1, 1, 576
        Hq, Hkv, Sk, Dh = 32, 16, 8192, 128
        assert Hq % Hkv == 0, (Hq, Hkv)
        return {
            "x": _w((lambda *s: _rng.normal(s) * 0.8)(B, Sq, D)),
            "k_cache": _w((lambda *s: _rng.normal(s) * 0.8)(B, Hkv, Sk, Dh)),
            "v_cache": _w((lambda *s: _rng.normal(s) * 0.05)(B, Hkv, Sk, Dh)),
            "wq": _w((lambda *s: _rng.normal(s) * 0.8)(D, Hq * Dh) * (D ** -0.5)),
            "wo": _w((lambda *s: _rng.normal(s) * 0.05)(Hq * Dh, D) * ((Hq * Dh) ** -0.5)),
        }
    _B_in = _B_setup()

    return {
        "A_x": _A_in["x"],
        "A_k_cache": _A_in["k_cache"],
        "A_v_cache": _A_in["v_cache"],
        "A_wq": _A_in["wq"],
        "A_wo": _A_in["wo"],
        "B_x": _B_in["x"],
        "B_k_cache": _B_in["k_cache"],
        "B_v_cache": _B_in["v_cache"],
        "B_wq": _B_in["wq"],
        "B_wo": _B_in["wo"],
    }

def reference(A_x, A_k_cache, A_v_cache, A_wq, A_wo, B_x, B_k_cache, B_v_cache, B_wq, B_wo):
    def _A_ref(x, k_cache, v_cache, wq, wo):
        B, Sq, D = x.shape
        Hq, Dh = 32, 128
        Hkv = k_cache.shape[1]
        rep = Hq // Hkv
        q = (lambda x, *d: x.transpose(*d))((x @ wq).reshape(B, Sq, Hq, Dh), 0, 2, 1, 3)
        k = jnp.repeat(k_cache, rep, axis=1)
        v = jnp.repeat(v_cache, rep, axis=1)
        scores = jnp.einsum("bhqd,bhkd->bhqk", q, k) * (Dh ** -0.5)
        p = _softmax(scores, axis=-1)
        o = jnp.einsum("bhqk,bhkd->bhqd", p, v)
        return (lambda x, *d: x.transpose(*d))(o, 0, 2, 1, 3).reshape(B, Sq, Hq * Dh) @ wo

    def _B_ref(x, k_cache, v_cache, wq, wo):
        B, Sq, D = x.shape
        Hq, Dh = 32, 128
        Hkv, Sk = k_cache.shape[1], k_cache.shape[2]
        W = min(4096, max(256, Sk // 4))
        rep = Hq // Hkv
        q = (lambda x, *d: x.transpose(*d))((x @ wq).reshape(B, Sq, Hq, Dh), 0, 2, 1, 3)
        k = jnp.repeat(k_cache[:, :, Sk - W:, :], rep, axis=1)
        v = jnp.repeat(v_cache[:, :, Sk - W:, :], rep, axis=1)
        scores = jnp.einsum("bhqd,bhkd->bhqk", q, k) * (Dh ** -0.5)
        p = _softmax(scores, axis=-1)
        o = jnp.einsum("bhqk,bhkd->bhqd", p, v)
        return (lambda x, *d: x.transpose(*d))(o, 0, 2, 1, 3).reshape(B, Sq, Hq * Dh) @ wo

    a = _A_ref(A_x, A_k_cache, A_v_cache, A_wq, A_wo)
    b = _B_ref(B_x, B_k_cache, B_v_cache, B_wq, B_wo)
    return jnp.concatenate([a, b], axis=-1)
```

```python
import functools
import jax
import jax.numpy as jnp
from jax import lax
from jax.experimental import pallas as pl
from jax.experimental.pallas import tpu as pltpu

D = 576
HQ, HKV, DH, SK = 32, 16, 128, 8192
WIN = 2048
NT = (((1,), (1,)), ((), ()))
F32, BF16 = jnp.float32, jnp.bfloat16


def build(ahead=2, prio=True, interleave="fine", compute=True, flags=None, name=None, nb_checks=True):
    G = 8
    nA, nB = SK // 128, WIN // 128
    phases = [("wqA", 9), ("wqB", 9), ("woB", 9), ("kA", nA), ("kB", nB), ("vB", nB), ("vA", nA), ("woA", 9)]
    starts = {}
    t = 0
    for n_, c_ in phases:
        starts[n_] = t
        t += c_
    total = t

    def locate(c):
        if c < 0 or c >= total:
            return None, 0
        for n_, c_ in phases:
            if c < starts[n_] + c_:
                return n_, c - starts[n_]

    def kernel(xA, kA, vA, wqA, woA, xB, kB, vB, wqB, woB, out_ref,
               x_buf, kA_buf, vA_buf, kB_buf, vB_buf, wqA_buf, wqB_buf, woA_buf, woB_buf,
               qA_ref, qB_ref, sA_ref, sB_ref, st_ref, oA_ref, oB_ref, sems, xsem):
        srcs = dict(wqA=(wqA, wqA_buf), wqB=(wqB, wqB_buf), woA=(woA, woA_buf), woB=(woB, woB_buf),
                    kA=(kA, kA_buf), vA=(vA, vA_buf), kB=(kB, kB_buf), vB=(vB, vB_buf))

        def views(ph, i, j, lo, n):
            src, dst = srcs[ph]
            half, quad = j // 4, j % 4
            if ph[0] == "w":
                r = i * 16 + half * 8
                if not isinstance(r, int):
                    r = pl.multiple_of(r, 8)
                idx = (pl.ds(lo, n), pl.ds(r, 8), pl.ds(quad * 1024, 1024))
                return src.at[idx], dst.at[idx]
            base = SK - WIN if ph[1] == "B" else 0
            r = base + i * 128 + half * 64
            if not isinstance(r, int):
                r = pl.multiple_of(r, 64)
            return (src.at[pl.ds(quad * 4 + lo, n), pl.ds(r, 64)],
                    dst.at[i, pl.ds(quad * 4 + lo, n), pl.ds(half * 64, 64)])

        def sem_of(ph, i, j):
            return sems.at[(starts[ph] + i) % ahead, j]

        def start(ph, i, j):
            if ph is None:
                return
            if prio:
                pltpu.make_async_copy(*views(ph, i, j, 0, 1), sem_of(ph, i, j)).start(priority=0)
                pltpu.make_async_copy(*views(ph, i, j, 1, 3), sem_of(ph, i, j)).start(priority=1)
            else:
                pltpu.make_async_copy(*views(ph, i, j, 0, 4), sem_of(ph, i, j)).start()

        def wait(ph, i, j):
            if ph is None:
                return
            pltpu.make_async_copy(*views(ph, i, j, 0, 4), sem_of(ph, i, j)).wait()

        row8 = lax.broadcasted_iota(jnp.int32, (8, 128), 0)

        def pick4(rs):
            r = rs[3]
            for g in (2, 1, 0):
                r = jnp.where(row8 < 2 * g + 2, rs[g], r)
            return r

        def q_block(which, hb):
            w = (wqA_buf, wqB_buf)[which]
            x = jnp.broadcast_to(x_buf[which, 0].astype(F32), (8, D)).astype(BF16)
            wv = w[:, :, hb * 1024:(hb + 1) * 1024].reshape(D, 1024)
            r = jnp.dot(x, wv, preferred_element_type=F32)
            q = r[:, 7 * 128:]
            for h in range(6, -1, -1):
                q = jnp.where(row8 <= h, r[:, h * 128:(h + 1) * 128], q)
            (qA_ref, qB_ref)[which][hb] = q

        def qk_piece(which, i, hb):
            k = (kA_buf, kB_buf)[which]
            q = (qA_ref, qB_ref)[which][hb].astype(BF16)
            s = pick4([lax.dot_general(q, k[i, 4 * hb + g], NT, preferred_element_type=F32) for g in range(4)])
            (sA_ref, sB_ref)[which][i, hb] = s
            st_ref[which, 0, hb] = jnp.maximum(st_ref[which, 0, hb], s)

        def pv_piece(which, i, hb):
            v = (vA_buf, vB_buf)[which]
            p = jnp.exp(((sA_ref, sB_ref)[which][i, hb] - st_ref[which, 0, hb]) * (DH ** -0.5))
            st_ref[which, 1, hb] += p
            pb = p.astype(BF16)
            st_ref[which, 2, hb] += pick4([jnp.dot(pb, v[i, 4 * hb + g], preferred_element_type=F32) for g in range(4)])

        def finish_max(which):
            for hb in range(4):
                m = jnp.max(st_ref[which, 0, hb], axis=1, keepdims=True)
                st_ref[which, 0, hb] = jnp.broadcast_to(m, (8, 128))

        def finish_o(which):
            o_ref = (oA_ref, oB_ref)[which]
            for hb in range(4):
                l = jnp.sum(st_ref[which, 1, hb], axis=1, keepdims=True)
                o = st_ref[which, 2, hb] / l
                for h in range(8):
                    o_ref[:, (8 * hb + h) * 128:(8 * hb + h + 1) * 128] = jnp.broadcast_to(o[h:h + 1], (8, 128))

        def out_block(which, hb):
            w = (woA_buf, woB_buf)[which]
            o = (oA_ref, oB_ref)[which][:, hb * 1024:(hb + 1) * 1024].astype(BF16)
            wv = w[:, :, hb * 1024:(hb + 1) * 1024].reshape(D, 1024)
            return lax.dot_general(o, wv, NT, preferred_element_type=F32)

        acc = {}

        def pieces(ph, i):
            if not compute or ph is None:
                return []
            if ph in ("kA", "kB"):
                return [functools.partial(qk_piece, int(ph[1] == "B"), i, hb) for hb in range(4)]
            if ph in ("vA", "vB"):
                return [functools.partial(pv_piece, int(ph[1] == "B"), i, hb) for hb in range(4)]
            if ph == "wqB" and i < 4:
                return [functools.partial(q_block, 0, i)]
            if ph == "woB" and i < 4:
                return [functools.partial(q_block, 1, i)]
            if ph == "woA" and i < 4:
                def f():
                    r = out_block(1, i)
                    acc["B"] = r if i == 0 else acc["B"] + r
                return [f]
            return []

        def step(cp, wt, st):
            ps = pieces(*cp)
            if interleave == "fine":
                for j in range(G):
                    wait(*wt, j)
                    start(*st, j)
                    if j % 2 == 0 and j // 2 < len(ps):
                        ps[j // 2]()
            else:
                for j in range(G):
                    wait(*wt, j)
                    start(*st, j)
                for p in ps:
                    p()

        for c in range(ahead):
            for j in range(G):
                start(*locate(c), j)
        xc = [pltpu.make_async_copy(x, x_buf.at[pl.ds(i, 1)], xsem.at[i]) for i, x in enumerate((xA, xB))]
        for c in xc:
            c.start()
        for w in range(2):
            st_ref[w, 0] = jnp.full((4, 8, 128), -jnp.inf, F32)
            st_ref[w, 1] = jnp.zeros((4, 8, 128), F32)
            st_ref[w, 2] = jnp.zeros((4, 8, 128), F32)

        c = 0
        while c < total:
            tri = [locate(c - 1), locate(c), locate(c + ahead)]
            n = 1
            if tri[0][0] is not None and tri[0][0][0] != "w":
                while all(locate(c + n + d)[0] == p[0] for d, p in zip((-1, 0, ahead), tri)):
                    n += 1
            if c == starts["wqB"]:
                for x in xc:
                    x.wait()
            if compute:
                if tri[0] == ("vB", 0):
                    finish_max(0)
                    finish_max(1)
                if tri[0] == ("woA", 0):
                    finish_o(0)
                    finish_o(1)
            if n == 1:
                step(*tri)
            else:
                def body(i, _, tri=tri):
                    step(*[(p, o + i) for p, o in tri])
                lax.fori_loop(0, n, body, None)
            c += n
        if compute:
            a = out_block(0, 0) + out_block(0, 1) + out_block(0, 2) + out_block(0, 3)
            out_ref[0] = jnp.concatenate([a[:1], acc["B"][:1]], axis=1).astype(BF16)
        else:
            out_ref[...] = jnp.zeros(out_ref.shape, BF16)

    def fn(A_x, A_k, A_v, A_wq, A_wo, B_x, B_k, B_v, B_wq, B_wo):
        w3 = lambda w: w.reshape(4, D // 4, HQ * DH)
        kv = lambda a: a.reshape(HKV, SK, DH)
        wbuf = pltpu.VMEM((4, D // 4, HQ * DH), BF16)
        return pl.pallas_call(
            kernel,
            in_specs=[pl.BlockSpec(memory_space=pl.ANY)] * 10,
            out_specs=pl.BlockSpec(memory_space=pltpu.VMEM),
            out_shape=jax.ShapeDtypeStruct((1, 1, 2 * D), BF16),
            scratch_shapes=[
                pltpu.VMEM((2, 1, D), BF16),
                pltpu.VMEM((nA, HKV, 128, DH), BF16), pltpu.VMEM((nA, HKV, 128, DH), BF16),
                pltpu.VMEM((nB, HKV, 128, DH), BF16), pltpu.VMEM((nB, HKV, 128, DH), BF16),
                wbuf, wbuf, wbuf, wbuf,
                pltpu.VMEM((4, 8, 128), F32), pltpu.VMEM((4, 8, 128), F32),
                pltpu.VMEM((nA, 4, 8, 128), F32), pltpu.VMEM((nB, 4, 8, 128), F32),
                pltpu.VMEM((2, 3, 4, 8, 128), F32),
                pltpu.VMEM((8, HQ * DH), F32), pltpu.VMEM((8, HQ * DH), F32),
                pltpu.SemaphoreType.DMA((ahead, G)), pltpu.SemaphoreType.DMA((2,)),
            ],
            compiler_params=pltpu.CompilerParams(vmem_limit_bytes=110 * 2**20, disable_bounds_checks=nb_checks, flags=flags),
            name=name,
        )(A_x, kv(A_k), kv(A_v), w3(A_wq), w3(A_wo.T), B_x, kv(B_k), kv(B_v), w3(B_wq), w3(B_wo.T))
    return fn


@jax.jit
def pallas_concat_heads__gqa_block_cached__sliding_block_cached__decode_kernel(
    A_x, A_k_cache, A_v_cache, A_wq, A_wo, B_x, B_k_cache, B_v_cache, B_wq, B_wo):
    return build()(A_x, A_k_cache, A_v_cache, A_wq, A_wo, B_x, B_k_cache, B_v_cache, B_wq, B_wo)
```

```python
import jax
import jax.numpy as jnp
from jax import lax
import jax.experimental.pallas as pl
import jax.experimental.pallas.tpu as pltpu

D, HQ, HKV, DH, SK = 576, 32, 16, 128, 8192
WIN = min(4096, max(256, SK // 4))
F32, BF16 = jnp.float32, jnp.bfloat16
NT = (((1,), (1,)), ((), ()))

SLAB = 64
NSLAB = D // SLAB
KEYS = 128
SLOTS = 8
AHEAD_LO = 4 * SLOTS
AHEAD_HI = 12
LAG = 4
RING = 16

N_A, N_B = SK // KEYS, WIN // KEYS
N_KV = N_A + N_B
N_WQ = 16
PHASES = (("wq", N_WQ), ("kA", N_A), ("kB", N_B), ("vA", N_A), ("vB", N_B))
WO_START = N_WQ + 2 * N_KV

ALL_SLABS = ((0, 1, 3), (4, 5, 4), (9, 10, 3), (13, 14, 4))


def _phase(chunk):
    first = 0
    for name, n in PHASES:
        if chunk < first + n:
            return name, first
        first += n
    return "wo", first


def _wo_plan():
    slots, blocks = [], {}

    def sweep(slabs, col0, ncol):
        for row in range(0, SLAB, 8):
            for col in range(col0, col0 + ncol, 1024):
                slots.extend((*s, row, 8, col, 1024) for s in slabs)

    def completes(*done):
        blocks[len(slots) - 1] = done

    sweep(ALL_SLABS, 0, 2048)
    completes(*[(0, 18, col, 512) for col in range(0, 2048, 512)])
    sweep(ALL_SLABS, 2048, 1024)
    completes((0, 18, 2048, 512), (0, 18, 2560, 512))
    sweep(((0, 1, 4), (9, 5, 4)), 3072, 1024)
    completes((0, 10, 3072, 1024))
    sweep(((10, 11, 3),), 3072, 1024)
    completes((10, 4, 3072, 1024))
    for first, col, ncol in ((14, 3072, 1024), (16, 3072, 512), (16, 3584, 512)):
        slots.append((None, first, 2, 0, SLAB, col, ncol))
        completes((first, 2, col, ncol))
    return slots, blocks


def _aligned(i, n):
    return i if isinstance(i, int) else pl.multiple_of(i, n)


def _attention_kernel(xA, kA, vA, wqA, woA, xB, kB, vB, wqB, woB, out_ref,
                      x_buf, kv_buf, wq_buf, wo_buf, q_ref, s_ref, m_ref, l_ref, acc_ref, o_ref,
                      *, sems, x_sems):
    wo_slots, wo_blocks = _wo_plan()

    def slot_spec(phase, chunk, j):
        name, first = phase
        i = chunk - first
        if name == "wo":
            hi, lo, n_lo, row, nrow, col, ncol = wo_slots[i * SLOTS + j]
            return wo_buf, hi, lo, n_lo, (pl.ds(row, nrow), pl.ds(col, ncol))
        if name == "wq":
            row = _aligned((i >> 1) * 8, 8)
            col = _aligned((2 * (i & 1) + j // 4) * 1024, 1024)
            return (wq_buf, *ALL_SLABS[j % 4], (pl.ds(row, 8), pl.ds(col, 1024)))
        head = 4 * (j % 4)
        return kv_buf.at[chunk & (RING - 1)], head, head + 1, 3, (pl.ds(64 * (j // 4), 64),)

    def slot_sem(chunk, j):
        return sems.at[chunk & (AHEAD_LO // SLOTS - 1), j]

    def start(phase, chunk, j, priority):
        name, first = phase
        if name == "wo" and (chunk - first) * SLOTS + j >= len(wo_slots):
            return
        buf, hi, lo, n_lo, rest = slot_spec(phase, chunk, j)
        lead, n = ((hi, 1), (lo, n_lo))[priority]
        if lead is None:
            return
        if name[0] == "w":
            src = {"wq": (wqA, wqB), "wo": (woA, woB)}[name][lead // NSLAB]
            src = src.at[(pl.ds(lead % NSLAB, n), *rest)]
        else:
            src, key0 = {"kA": (kA, 0), "vA": (vA, 0), "kB": (kB, SK - WIN), "vB": (vB, SK - WIN)}[name]
            key = key0 + (chunk - first) * KEYS + 64 * (j // 4)
            src = src.at[pl.ds(lead, n), pl.ds(_aligned(key, 64), 64)]
        dst = buf.at[(pl.ds(lead, n), *rest)]
        pltpu.make_async_copy(src, dst, slot_sem(chunk, j)).start(priority=priority)

    def wait(phase, chunk, j):
        buf, hi, lo, n_lo, rest = slot_spec(phase, chunk, j)
        lead = pl.ds(lo, n_lo) if hi is None else pl.ds(min(hi, lo), n_lo + 1)
        dst = buf.at[(lead, *rest)]
        pltpu.make_async_copy(dst, dst, slot_sem(chunk, j)).wait()

    def advance(chunk0, chunk, j):
        wait(_phase(chunk0), chunk, j)
        for priority, ahead in enumerate((AHEAD_HI, AHEAD_LO)):
            d, k = divmod(j + ahead, SLOTS)
            start(_phase(chunk0 + d), chunk + d, k, priority)

    sublane = lax.broadcasted_iota(jnp.int32, (8, 128), 0)
    lane = lax.broadcasted_iota(jnp.int32, (8, 128), 1)

    def own_rows(per_kv_head):
        r = per_kv_head[3]
        for g in (2, 1, 0):
            r = jnp.where(sublane < 2 * g + 2, per_kv_head[g], r)
        return r

    def project_q(block, quad):
        x = jnp.broadcast_to(x_buf[block].astype(F32), (8, D)).astype(BF16)
        w = wq_buf[pl.ds(block * NSLAB, NSLAB), :, pl.ds(_aligned(quad * 512, 512), 512)]
        q = jnp.dot(x, w.reshape(D, 512), preferred_element_type=F32)
        for h in range(4):
            q_ref[block, pl.ds(4 * quad + h, 1), :] = q[:1, h * DH:(h + 1) * DH]

    def scores(block, i, ring, hb):
        q = q_ref[block, 8 * hb:8 * hb + 8].astype(BF16)
        s = own_rows([lax.dot_general(q, kv_buf[ring, 4 * hb + g], NT, preferred_element_type=F32)
                      for g in range(4)]) * (DH ** -0.5)
        s_ref[i, hb] = s
        m_ref[block, hb] = jnp.maximum(m_ref[block, hb], s)

    def weighted_values(block, i, ring, hb):
        p = jnp.exp(s_ref[i, hb] - m_ref[block, hb])
        l_ref[block, hb] += p
        p = p.astype(BF16)
        acc_ref[block, hb] += own_rows([jnp.dot(p, kv_buf[ring, 4 * hb + g], preferred_element_type=F32)
                                        for g in range(4)])

    def work_kind(chunk):
        i = chunk - N_WQ - LAG
        return None if chunk < N_WQ else "q" if i < 0 else "qk" if i < N_KV else "pv"

    def stream_chunk(chunk0, chunk):
        kind = work_kind(chunk0)
        for j in range(SLOTS):
            advance(chunk0, chunk, j)
            if kind is None or j % 2:
                continue
            piece = j // 2
            if kind == "q":
                project_q(piece % 2, 2 * (chunk - N_WQ) + piece // 2)
                continue
            i = chunk - N_WQ - LAG - (N_KV if kind == "pv" else 0)
            block = int(i >= N_A) if isinstance(i, int) else (i >= N_A).astype(jnp.int32)
            (scores if kind == "qk" else weighted_values)(block, i, (chunk - LAG) & (RING - 1), piece)

    for t in range(AHEAD_LO):
        chunk, j = divmod(t, SLOTS)
        if t < AHEAD_HI:
            start(_phase(chunk), chunk, j, 0)
        start(_phase(chunk), chunk, j, 1)
    x_copies = [pltpu.make_async_copy(x, x_buf.at[pl.ds(b, 1)], x_sems.at[b]) for b, x in enumerate((xA, xB))]
    for c in x_copies:
        c.start()
    m_ref[...] = jnp.full(m_ref.shape, -jnp.inf, F32)
    l_ref[...] = jnp.zeros(l_ref.shape, F32)
    acc_ref[...] = jnp.zeros(acc_ref.shape, F32)

    def signature(chunk):
        ahead = (AHEAD_HI // SLOTS, (AHEAD_HI + SLOTS - 1) // SLOTS, AHEAD_LO // SLOTS)
        return (work_kind(chunk), *[_phase(chunk + d)[0] for d in ahead])

    chunk0 = 0
    while chunk0 < WO_START + LAG:
        if chunk0 == N_WQ:
            for c in x_copies:
                c.wait()
        if chunk0 == N_WQ + LAG + N_KV:
            for b in range(2):
                for hb in range(4):
                    m_ref[b, hb] = jnp.broadcast_to(jnp.max(m_ref[b, hb], axis=1, keepdims=True), (8, 128))
        n = 1
        while signature(chunk0)[-1] != "wo" and signature(chunk0 + n) == signature(chunk0):
            n += 1
        if n == 1:
            stream_chunk(chunk0, chunk0)
        else:
            lax.fori_loop(chunk0, chunk0 + n, lambda c, _, c0=chunk0: stream_chunk(c0, c), None)
        chunk0 += n

    for hb in range(4):
        o = [acc_ref[b, hb] / jnp.sum(l_ref[b, hb], axis=1, keepdims=True) for b in range(2)]
        for h in range(8):
            rows = jnp.concatenate([jnp.broadcast_to(x[h:h + 1], (8, DH)) for x in o], axis=0)
            o_ref[:, (8 * hb + h) * DH:(8 * hb + h + 1) * DH] = rows.astype(BF16)

    out_tiles = [None] * (2 * D // 128)

    def project_out(first, nslab, col, ncol):
        w = wo_buf[first:first + nslab, :, col:col + ncol].reshape(nslab * SLAB, ncol)
        r = lax.dot_general(o_ref[:, col:col + ncol], w, NT, preferred_element_type=F32)
        for u in range(nslab * SLAB // 128):
            t = first * SLAB // 128 + u
            a, b = r[:8, u * 128:(u + 1) * 128], r[8:, u * 128:(u + 1) * 128]
            n_a = D - 128 * t
            part = a if n_a >= 128 else b if n_a <= 0 else jnp.where(lane < n_a, a, b)
            out_tiles[t] = part if out_tiles[t] is None else out_tiles[t] + part

    ready, due = [], 0
    for t in range(LAG * SLOTS, len(wo_slots)):
        chunk = WO_START + t // SLOTS
        advance(chunk, chunk, t % SLOTS)
        if t in wo_blocks:
            ready.extend(wo_blocks[t])
            due = t
        if ready and t >= due:
            project_out(*ready.pop(0))
            due = t + SLOTS - 1
    assert not ready
    out_ref[0] = jnp.concatenate(out_tiles, axis=1)[:1].astype(out_ref.dtype)


def _kernel(*refs):
    pl.run_scoped(
        lambda sems, x_sems: _attention_kernel(*refs, sems=sems, x_sems=x_sems),
        pltpu.SemaphoreType.DMA((AHEAD_LO // SLOTS, SLOTS)),
        pltpu.SemaphoreType.DMA((2,)),
    )


@jax.jit
def pallas_concat_heads__gqa_block_cached__sliding_block_cached__decode_kernel(
    A_x: jax.Array,
    A_k_cache: jax.Array,
    A_v_cache: jax.Array,
    A_wq: jax.Array,
    A_wo: jax.Array,
    B_x: jax.Array,
    B_k_cache: jax.Array,
    B_v_cache: jax.Array,
    B_wq: jax.Array,
    B_wo: jax.Array,
):
    heads = lambda a: a.reshape(HKV, SK, DH)
    slabs = lambda w: w.reshape(NSLAB, SLAB, HQ * DH)
    stat = pltpu.VMEM((2, 4, 8, 128), F32)
    return pl.pallas_call(
        _kernel,
        in_specs=[pl.BlockSpec(memory_space=pltpu.MemorySpace.HBM)] * 10,
        out_specs=pl.BlockSpec(memory_space=pltpu.MemorySpace.VMEM),
        out_shape=jax.ShapeDtypeStruct((1, 1, 2 * D), A_x.dtype),
        scratch_shapes=[
            pltpu.VMEM((2, 1, D), BF16),
            pltpu.VMEM((RING, HKV, KEYS, DH), BF16),
            pltpu.VMEM((2 * NSLAB, SLAB, HQ * DH), BF16),
            pltpu.VMEM((2 * NSLAB, SLAB, HQ * DH), BF16),
            pltpu.VMEM((2, HQ, DH), F32),
            pltpu.VMEM((N_KV, 4, 8, KEYS), F32),
            stat, stat, stat,
            pltpu.VMEM((16, HQ * DH), BF16),
        ],
        compiler_params=pltpu.CompilerParams(vmem_limit_bytes=48 * 2**20),
    )(A_x, heads(A_k_cache), heads(A_v_cache), slabs(A_wq), slabs(A_wo.T),
      B_x, heads(B_k_cache), heads(B_v_cache), slabs(B_wq), slabs(B_wo.T))
```
